```python
import os as _os
_os.environ.setdefault("JAX_PLATFORMS", "cpu")
import jax
import jax.numpy as jnp

def _softmax(x, axis=-1):
    return jax.nn.softmax(x, axis=axis)
def _gelu(x):
    return jax.nn.gelu(x, approximate=True)
def _silu(x):
    return jax.nn.silu(x)
def _sigmoid(x):
    return jax.nn.sigmoid(x)
def _layernorm(x, axis=-1, eps=1e-5):
    m = jnp.mean(x, axis=axis, keepdims=True)
    v = jnp.var(x, axis=axis, keepdims=True)
    return (x - m) / jnp.sqrt(v + eps)
def _scatter_add(tgt, idx, src, axis=0):
    return tgt.at[idx].add(src)
def _segment_sum(src, seg, n):
    return jax.ops.segment_sum(src, seg, n)
class _Rng:
    def __init__(self, key):
        self._k = key
    def _next(self):
        self._k, sub = jax.random.split(self._k)
        return sub
    def normal(self, shape):
        return jax.random.normal(self._next(), shape, dtype=jnp.bfloat16)
    def randint(self, lo, hi, shape):
        return jax.random.randint(self._next(), shape, lo, hi, dtype=jnp.int32)
    def uniform(self, shape, lo=0.0, hi=1.0):
        return jax.random.uniform(self._next(), shape, jnp.bfloat16, lo, hi)
    def permutation(self, n):
        return jax.random.permutation(self._next(), n)


kernel_name = 'gated_mix__compressed_kv_cla__linear_attn_block__prompt'

def setup_inputs():
    _rng = _Rng(jax.random.key(int.from_bytes(__import__("os").urandom(4), "little")))
    _w = (lambda a: (lambda t: t.astype(jnp.bfloat16) if jnp.issubdtype(t.dtype, jnp.floating) else t)(jnp.asarray(a)))
    def _A_setup():
        B, H, Sq, Sk, D, M = 1, 16, 2048, 2048, 256, 448
        Dc = 4 * D
        return {
            "x": _w((lambda *s: _rng.normal(s) * 0.05)(B, Sq, M)),
            "c_kv": _w((lambda *s: _rng.normal(s) * 0.8)(B, Sk, Dc)),
            "w_q": _w((lambda *s: _rng.normal(s) * 3.2)(M, H, D) * (M ** -0.5)),
            "w_uk": _w((lambda *s: _rng.normal(s) * 3.2)(Dc, H, D) * (Dc ** -0.5)),
            "w_uv": _w((lambda *s: _rng.normal(s) * 0.8)(Dc, H, D) * (Dc ** -0.5)),
            "w_o": _w((lambda *s: _rng.normal(s) * 0.8)(H, D, M) * ((H * D) ** -0.5)),
        }
    _A_in = _A_setup()

    def _B_setup():
        B, S, D = 1, 2048, 448
        return {
            "x": _w((lambda *s: _rng.normal(s) * 0.05)(B, S, D)),
            "wqkv": _w((lambda *s: _rng.normal(s) * 1.6)(D, 3 * D)),
            "wo": _w((lambda *s: _rng.normal(s) * 0.4)(D, D)),
        }
    _B_in = _B_setup()

    return {
        "A_x": _A_in["x"],
        "A_c_kv": _A_in["c_kv"],
        "A_w_q": _A_in["w_q"],
        "A_w_uk": _A_in["w_uk"],
        "A_w_uv": _A_in["w_uv"],
        "A_w_o": _A_in["w_o"],
        "B_x": _B_in["x"],
        "B_wqkv": _B_in["wqkv"],
        "B_wo": _B_in["wo"],
        "gate_w": _w((lambda *s: _rng.normal(s) * 0.05)(448) * 16.0),
    }

def reference(A_x, A_c_kv, A_w_q, A_w_uk, A_w_uv, A_w_o, B_x, B_wqkv, B_wo, gate_w):
    def _A_ref(x, c_kv, w_q, w_uk, w_uv, w_o):
        B, Sq, M = x.shape[0], x.shape[1], x.shape[2]
        Sk = c_kv.shape[1]
        H, D = w_q.shape[1], w_q.shape[2]
        q = jnp.einsum("bqm,mhd->bhqd", x, w_q)
        k = jnp.einsum("bkc,chd->bhkd", c_kv, w_uk)
        v = jnp.einsum("bkc,chd->bhkd", c_kv, w_uv)
        scores = jnp.einsum("bhqd,bhkd->bhqk", q, k) * (D ** -0.5)
        off = Sk - Sq
        qi = jnp.arange(Sq)[:, None]
        kj = jnp.arange(Sk)[None, :]
        cmask = kj <= (qi + off)
        scores = jnp.where(cmask[None, None], scores, -1e9)
        p = _softmax(scores, axis=-1)
        ctx = jnp.einsum("bhqk,bhkd->bhqd", p, v)
        return jnp.einsum("bhqd,hdm->bqm", ctx, w_o)

    def _B_ref(x, wqkv, wo):
        B, S, D = x.shape
        H = 16; Dh = D // H
        qkv = (lambda x, *d: x.transpose(*d))((x @ wqkv).reshape(B, S, 3, H, Dh), 2, 0, 3, 1, 4)
        q, k, v = qkv[0], qkv[1], qkv[2]
        phi = lambda t: jnp.where(t > 0, t + 1, jnp.exp(t)) + 1e-6
        pq, pk = phi(q), phi(k)
        kv = jnp.einsum("bhsd,bhse->bhde", pk, v)
        z = jnp.einsum("bhsd->bhd", pk)
        num = jnp.einsum("bhqd,bhde->bhqe", pq, kv)
        den = jnp.einsum("bhqd,bhd->bhq", pq, z)[..., None] + 1e-6
        o = num / den
        return (lambda x, *d: x.transpose(*d))(o, 0, 2, 1, 3).reshape(B, S, D) @ wo

    x = A_x
    g = _sigmoid((x * gate_w).sum(-1, keepdims=True))
    a = _A_ref(x, A_c_kv, A_w_q, A_w_uk, A_w_uv, A_w_o)
    b = _B_ref(x, B_wqkv, B_wo)
    return g * a + (1 - g) * b
```

```python
import os
import functools
import jax
import jax.numpy as jnp
from jax import lax
import jax.experimental.pallas as pl
import jax.experimental.pallas.tpu as pltpu

NT = (((1,), (1,)), ((), ()))
NN = (((1,), (0,)), ((), ()))
LOG2E = 1.4426950408889634
BQ = 256
F32 = jnp.float32
BF = jnp.bfloat16
DIAG = 1
PACE = int(os.environ.get("PACE", "2"))
LBF = int(os.environ.get("LBF", "1"))

ERANGE = ((0, 144), (112, 288), (240, 400), (352, 448))


def _deint_piece(dst_ref, raw_ref, u, j, m0, nm):
    r32 = raw_ref.bitcast(jnp.uint32)
    w = r32[pl.ds(j, nm, stride=8), :]
    dst_ref[2 * j, pl.ds(m0, nm), u * 128:(u + 1) * 128] = pltpu.bitcast(w << 16, F32).astype(BF)
    dst_ref[2 * j + 1, pl.ds(m0, nm), u * 128:(u + 1) * 128] = pltpu.bitcast(w & jnp.uint32(0xFFFF0000), F32).astype(BF)


def kernel(xT_hbm, c_hbm, wq_hbm, wk_hbm, wv_hbm, woT_hbm, wqkv_hbm, bwo_hbm, gw_ref,
           out_hbm,
           xT_s, c_s, wq_r, wk_r, wv_r, woT_s, wqkv_s, bwo_s, out_s,
           q_all, k_s, v_s, s_s, acc_s, bT_s, g_s, wq_d, wk_d, wv_d, xa_s, wqkvT_s, pqT_s, bwoT_s, kv_s, kvm_s, zm_s,
           sems, csems, osems, xsems):
    M, S = xT_s.shape
    D = 256
    H = 16
    NB = S // BQ

    cp_wqkv = pltpu.make_async_copy(wqkv_hbm, wqkv_s, sems.at[1])
    cp_bwo = pltpu.make_async_copy(bwo_hbm, bwo_s, sems.at[2])
    cp_wq = [pltpu.make_async_copy(wq_hbm.at[:, pl.ds(128 * u, 128)], wq_r.at[u], sems.at[3 + u]) for u in range(2)]
    cp_c = pltpu.make_async_copy(c_hbm.at[0], c_s, sems.at[5])
    cp_wo = pltpu.make_async_copy(woT_hbm, woT_s, sems.at[6])

    def cp_kv(i, which, u):
        src = (wk_hbm, wv_hbm)[which]
        dst = (wk_r, wv_r)[which]
        return pltpu.make_async_copy(src.at[pl.ds(i * 1024, 1024), pl.ds(128 * u, 128)], dst.at[u, i], csems.at[i, 2 * which + u])

    NX = 4
    XW = S // NX
    cp_x = [pltpu.make_async_copy(xT_hbm.at[0, :, pl.ds(i * XW, XW)], xT_s.at[:, pl.ds(i * XW, XW)], xsems.at[i]) for i in range(NX)]
    cp_wqkv.start(); cp_x[0].start()

    def start_kv(lo, hi):
        for i in range(lo, hi):
            for w in range(2):
                for u in range(2):
                    cp_kv(i, w, u).start()

    with jax.named_scope("w_wqkv"):
        cp_wqkv.wait()
    for i in range(1, NX):
        cp_x[i].start()
    cp_bwo.start()
    for u in range(11):
        w = min(128, 1344 - u * 128)
        wqkvT_s[u*128:u*128+w, :] = wqkv_s[:, u*128:u*128+w].astype(F32).T.astype(BF)
    wqkvT_s[1344:1360, :] = jnp.broadcast_to(gw_ref[...], (16, M)).astype(BF)
    with jax.named_scope("w_x"):
        cp_x[0].wait()
    cp_wq[0].start(); cp_wq[1].start()
    CH = int(os.environ.get('CH1', '512'))
    NC = S // CH
    kv_s[...] = jnp.zeros_like(kv_s)

    def p1body(i, _, deint):
        @pl.when(i == 1)
        def _():
            cp_bwo.wait()
            bwoT_s[...] = bwo_s[...].astype(F32).T.astype(BF)
        for n in range(1, NX):
            @pl.when(i == n * (XW // CH))
            def _():
                cp_x[n].wait()
        @pl.when(i == NC * 3 // 4)
        def _():
            start_kv(4, 8)
        cols = pl.ds(pl.multiple_of(i * CH, CH), CH)
        xb = xT_s[:, cols]
        t = jnp.dot(wqkvT_s[0:896, :], xb, preferred_element_type=F32)
        ph = (jnp.where(t > 0, t + 1.0, jnp.exp(t)) + 1e-6).astype(BF)
        pqT_s[:, cols] = ph[0:448]
        vg = jnp.dot(wqkvT_s[896:1360, :], xb, preferred_element_type=F32)
        vT = vg[0:448].astype(BF)
        g_s[:, cols] = 1.0 / (1.0 + jnp.exp(-vg[448:456]))
        ones = jnp.ones((16, CH), BF)
        for r, (lo, hi) in enumerate(ERANGE):
            dn = min(128, 448 - 128 * r)
            lhs = jnp.concatenate([vT[lo:hi], ones], axis=0)
            kk = lax.dot_general(lhs, ph[448 + 128 * r:448 + 128 * r + dn], NT, preferred_element_type=F32)
            kv_s[r, 0:hi - lo + 16, 0:dn] += kk
        xa_s[cols, :] = xb.astype(F32).T.astype(BF)
        acc_s[:, cols] = jnp.zeros((M, CH), F32)
        if deint:
            per = 8 // NC
            for e in range(per):
                mc = (i - NC // 2) * per + e
                for u in range(2):
                    sub = wq_r.at[u, pl.ds(pl.multiple_of(mc * 1792, 1792), 1792)]
                    for j in range(8):
                        _deint_piece(wq_d, sub, u, j, pl.multiple_of(mc * 112, 16), 112)
        return _
    with jax.named_scope("pass1"):
        lax.fori_loop(0, NC // 2, functools.partial(p1body, deint=False), None)
    with jax.named_scope("w_wq"):
        cp_wq[0].wait(); cp_wq[1].wait()
    start_kv(0, 4)
    with jax.named_scope("pass1b"):
        lax.fori_loop(NC // 2, NC, functools.partial(p1body, deint=True), None)

    for r, (lo, hi) in enumerate(ERANGE):
        dn = min(128, 448 - 128 * r)
        n = hi - lo
        e = lax.broadcasted_iota(jnp.int32, (n, dn), 0) + lo
        d = lax.broadcasted_iota(jnp.int32, (n, dn), 1) + 128 * r
        same = ((e * 2341) >> 16) == ((d * 2341) >> 16)
        kvm_s[r, 0:n, 0:dn] = jnp.where(same, kv_s[r, 0:n, 0:dn], 0.0).astype(BF)
        zrow = kv_s[r, n:n + 8, 0:dn]
        zm_s[r, 0:n, 0:dn] = jnp.where(same, jnp.tile(zrow, (n // 8, 1)), 0.0).astype(BF)

    def assemble(parts):
        out = []
        bounds = sorted(set([0, 448] + [x for rg in ERANGE for x in rg]))
        for a, b in zip(bounds[:-1], bounds[1:]):
            acc = None
            for r, (lo, hi) in enumerate(ERANGE):
                if lo <= a and b <= hi:
                    p = parts[r][a - lo:b - lo]
                    acc = p if acc is None else acc + p
            out.append(acc)
        return jnp.concatenate(out, axis=0)

    def numden(i):
        cols = pl.ds(pl.multiple_of(i * CH, CH), CH)
        nums = []; dens = []
        for r, (lo, hi) in enumerate(ERANGE):
            dn = min(128, 448 - 128 * r)
            pq = pqT_s[128 * r:128 * r + dn, cols]
            nums.append(jnp.dot(kvm_s[r, 0:hi - lo, 0:dn], pq, preferred_element_type=F32))
            dens.append(jnp.dot(zm_s[r, 0:hi - lo, 0:dn], pq, preferred_element_type=F32))
        return (assemble(nums) / (assemble(dens) + 1e-6)).astype(BF)

    CH = 256
    NC = S // CH
    start_kv(8, 12)

    def p2body(i, _):
        @pl.when(i == 2)
        def _():
            start_kv(12, 16)
        oa = numden(2 * i)
        ob = numden(2 * i + 1)
        for n, o in enumerate((oa, ob)):
            cols = pl.ds(pl.multiple_of((2 * i + n) * CH, CH), CH)
            bT_s[:, cols] = (1.0 - g_s[0:1, cols]) * jnp.dot(bwoT_s[...], o, preferred_element_type=F32)
        return _
    with jax.named_scope("pass2"):
        lax.fori_loop(0, NC // 2, p2body, None)

    def qbody(h, _):
        m0 = pl.multiple_of(h * 64, 64)
        wq = wq_d[h]
        for i in range(S // 256):
            rows = slice(i * 256, (i + 1) * 256)
            q_all[h, rows, :] = (jnp.dot(xa_s[rows, :], wq, preferred_element_type=F32) * (LOG2E / 16.0)).astype(BF)
            for u in range(2):
                _deint_piece(wk_d, wk_r.at[u, h], u, i, m0, 64)
                _deint_piece(wv_d, wv_r.at[u, h], u, i, m0, 64)
        return _
    for half in range(2):
        with jax.named_scope("w_kv%d" % half):
            for i in range(half * 8, half * 8 + 8):
                for w in range(2):
                    for u in range(2):
                        cp_kv(i, w, u).wait()
        (cp_c, cp_wo)[half].start()
        with jax.named_scope("qloop%d" % half):
            lax.fori_loop(half * 8, half * 8 + 8, qbody, None)

    with jax.named_scope("w_c"):
        cp_c.wait(); cp_wo.wait()

    def outproj(hh, t, ctx):
        acc_s[:, t * BQ:(t + 1) * BQ] += lax.dot_general(woT_s[hh], ctx, NT, preferred_element_type=F32)

    def kproj(hh, i):
        rows = slice(i * BQ, (i + 1) * BQ)
        k_s[rows, :] = jnp.dot(c_s[rows, :], wk_d[hh], preferred_element_type=F32).astype(BF)

    def vproj(hh, i):
        rows = slice(i * BQ, (i + 1) * BQ)
        v_s[rows, :] = jnp.dot(c_s[rows, :], wv_d[hh], preferred_element_type=F32).astype(BF)

    def hbody(h, _):
        HB = BQ // 2
        tri = lax.broadcasted_iota(jnp.int32, (HB, HB), 1) <= lax.broadcasted_iota(jnp.int32, (HB, HB), 0)

        def qk(t):
            q = q_all[h, t * BQ:(t + 1) * BQ, :]
            m = None
            sl = t % 2
            for j in range(t):
                s = lax.dot_general(q, k_s[j * BQ:(j + 1) * BQ, :], NT, preferred_element_type=F32)
                s_s[sl, :, j * BQ:(j + 1) * BQ] = s
                for u in range(BQ // 128):
                    mm = s[:, u * 128:(u + 1) * 128]
                    m = mm if m is None else jnp.maximum(m, mm)
            c0 = t * BQ
            if DIAG == 0:
                s = lax.dot_general(q, k_s[c0:c0 + BQ, :], NT, preferred_element_type=F32)
                r = lax.broadcasted_iota(jnp.int32, (BQ, BQ), 1)
                c = lax.broadcasted_iota(jnp.int32, (BQ, BQ), 0)
                s = jnp.where(r <= c, s, -1e9)
                s_s[sl, :, c0:c0 + BQ] = s
                for u in range(BQ // 128):
                    mm = s[:, u * 128:(u + 1) * 128]
                    m = mm if m is None else jnp.maximum(m, mm)
                return jnp.max(m, axis=1, keepdims=True)
            else:
                sa = lax.dot_general(q, k_s[c0:c0 + HB, :], NT, preferred_element_type=F32)
                sb = lax.dot_general(q[HB:], k_s[c0 + HB:c0 + BQ, :], NT, preferred_element_type=F32)
                sa = jnp.concatenate([jnp.where(tri, sa[:HB], -1e9), sa[HB:]], axis=0)
                sb = jnp.where(tri, sb, -1e9)
                s_s[sl, :, c0:c0 + HB] = sa
                s_s[sl, HB:, c0 + HB:c0 + BQ] = sb
                m = sa if m is None else jnp.maximum(m, sa)
                m = jnp.concatenate([m[:HB], jnp.maximum(m[HB:], sb)], axis=0)
                return jnp.max(m, axis=1, keepdims=True)

        def pv(t, m):
            acc = None; l = None
            sl = t % 2
            prev = []
            def paced(mm):
                if PACE and len(prev) >= PACE:
                    a = prev[-PACE][:, 0:1]
                    return jnp.maximum(mm, jnp.minimum(mm, a))
                return mm
            def psum(p):
                pb = p.astype(BF)
                return pb, (pb.astype(F32) if LBF else p)
            for j in range(t):
                p = jnp.exp2(s_s[sl, :, j * BQ:(j + 1) * BQ] - paced(m))
                pb, p = psum(p)
                for u in range(BQ // 128):
                    ll = p[:, u * 128:(u + 1) * 128]
                    l = ll if l is None else l + ll
                a = jnp.dot(pb, v_s[j * BQ:(j + 1) * BQ, :], preferred_element_type=F32)
                prev.append(a)
                acc = a if acc is None else acc + a
            c0 = t * BQ
            mm = paced(m)
            pa, paf = psum(jnp.exp2(s_s[sl, :, c0:c0 + HB] - mm))
            pb, pbf = psum(jnp.exp2(s_s[sl, HB:, c0 + HB:c0 + BQ] - mm[HB:]))
            l = paf if l is None else l + paf
            l = jnp.concatenate([l[:HB], l[HB:] + pbf], axis=0)
            a = jnp.dot(pa, v_s[c0:c0 + HB, :], preferred_element_type=F32)
            acc = a if acc is None else acc + a
            a2 = jnp.dot(pb, v_s[c0 + HB:c0 + BQ, :], preferred_element_type=F32)
            acc = jnp.concatenate([acc[:HB], acc[HB:] + a2], axis=0)
            l = jnp.sum(l, axis=1, keepdims=True)
            return (acc * (1.0 / l)).astype(BF)

        hn = jnp.minimum(h + 1, H - 1)
        for t in range(NB):
            m = qk(t)
            if t + 1 < NB:
                kproj(h, t + 1)
            else:
                kproj(hn, 0)
            ctx = pv(t, m)
            if t + 1 < NB:
                vproj(h, t + 1)
            else:
                vproj(hn, 0)
            outproj(h, t, ctx)
        return _
    with jax.named_scope("hloop"):
        kproj(0, 0); vproj(0, 0)
        lax.fori_loop(0, H, hbody, None)

    NO = 4
    W = S // NO
    ocp = []
    for i in range(NO):
        cols = slice(i * W, (i + 1) * W)
        out_s[:, cols] = (g_s[0:1, cols] * acc_s[:, cols] + bT_s[:, cols]).astype(out_s.dtype)
        cp = pltpu.make_async_copy(out_s.at[:, pl.ds(i * W, W)], out_hbm.at[0, :, pl.ds(i * W, W)], osems.at[i])
        cp.start()
        ocp.append(cp)
    with jax.named_scope("w_out"):
        for cp in ocp:
            cp.wait()


@jax.jit
def pallas_gated_mix__compressed_kv_cla__linear_attn_block__prompt_kernel(
    A_x, A_c_kv, A_w_q, A_w_uk, A_w_uv, A_w_o, B_x, B_wqkv, B_wo, gate_w,
):
    B, S, M = A_x.shape
    Dc = A_c_kv.shape[2]
    H, D = A_w_q.shape[1], A_w_q.shape[2]
    anyspec = pl.BlockSpec(memory_space=pl.ANY)
    wq = A_w_q.reshape(M * H, D)
    wk = A_w_uk.reshape(Dc * H, D)
    wv = A_w_uv.reshape(Dc * H, D)
    outT = pl.pallas_call(
        kernel,
        in_specs=[anyspec] * 8 + [pl.BlockSpec(memory_space=pltpu.VMEM)],
        out_specs=anyspec,
        out_shape=jax.ShapeDtypeStruct((B, M, S), BF),
        scratch_shapes=[
            pltpu.VMEM((M, S), BF), pltpu.VMEM((S, Dc), BF), pltpu.VMEM((2, M * H, 128), BF),
            pltpu.VMEM((2, H, Dc, 128), BF), pltpu.VMEM((2, H, Dc, 128), BF), pltpu.VMEM((H, M, D), BF),
            pltpu.VMEM((M, 3 * M), BF), pltpu.VMEM((M, M), BF), pltpu.VMEM((M, S), BF),
            pltpu.VMEM((H, S, D), BF), pltpu.VMEM((S, D), BF), pltpu.VMEM((S, D), BF),
            pltpu.VMEM((2, BQ, S), F32), pltpu.VMEM((M, S), F32), pltpu.VMEM((M, S), F32), pltpu.VMEM((8, S), F32),
            pltpu.VMEM((H, M, D), BF), pltpu.VMEM((H, Dc, D), BF), pltpu.VMEM((H, Dc, D), BF),
            pltpu.VMEM((S, M), BF), pltpu.VMEM((3 * M + 16, M), BF), pltpu.VMEM((M, S), BF), pltpu.VMEM((M, M), BF),
            pltpu.VMEM((4, 192, 128), F32), pltpu.VMEM((4, 176, 128), BF), pltpu.VMEM((4, 176, 128), BF),
            pltpu.SemaphoreType.DMA((7,)), pltpu.SemaphoreType.DMA((H, 4)), pltpu.SemaphoreType.DMA((4,)), pltpu.SemaphoreType.DMA((4,)),
        ],
        compiler_params=pltpu.CompilerParams(vmem_limit_bytes=120 * 2**20),
    )(A_x.transpose(0, 2, 1), A_c_kv, wq, wk, wv, A_w_o.transpose(0, 2, 1), B_wqkv, B_wo, gate_w.reshape(1, M))
    return outT.transpose(0, 2, 1)
```

```python
import functools
import jax
import jax.numpy as jnp
from jax import lax
import jax.experimental.pallas as pl
import jax.experimental.pallas.tpu as pltpu

NT = (((1,), (1,)), ((), ()))
NN = (((1,), (0,)), ((), ()))
LOG2E = 1.4426950408889634
BQ = 256
F32 = jnp.float32
BF = jnp.bfloat16
DIAG = 1
PACE = 2
LBF = 1

ERANGE = ((0, 144), (112, 288), (240, 400), (352, 448))


def _deint_piece(dst_ref, raw_ref, u, j, m0, nm):
    r32 = raw_ref.bitcast(jnp.uint32)
    w = r32[pl.ds(j, nm, stride=8), :]
    dst_ref[2 * j, pl.ds(m0, nm), u * 128:(u + 1) * 128] = pltpu.bitcast(w << 16, F32).astype(BF)
    dst_ref[2 * j + 1, pl.ds(m0, nm), u * 128:(u + 1) * 128] = pltpu.bitcast(w & jnp.uint32(0xFFFF0000), F32).astype(BF)


def kernel(xT_hbm, c_hbm, wq_hbm, wk_hbm, wv_hbm, woT_hbm, wqkv_hbm, bwo_hbm, gw_ref,
           out_hbm,
           xT_s, c_s, wq_r, wk_r, wv_r, woT_s, wqkv_s, bwo_s, out_s,
           q_all, k_s, v_s, s_s, acc_s, bT_s, g_s, wq_d, wk_d, wv_d, xa_s, wqkvT_s, pqT_s, bwoT_s, kv_s, kvm_s, zm_s,
           sems, csems, osems, xsems):
    M, S = xT_s.shape
    D = 256
    H = 16
    NB = S // BQ

    cp_wqkv = pltpu.make_async_copy(wqkv_hbm, wqkv_s, sems.at[1])
    cp_bwo = pltpu.make_async_copy(bwo_hbm, bwo_s, sems.at[2])
    cp_wq = [pltpu.make_async_copy(wq_hbm.at[:, pl.ds(128 * u, 128)], wq_r.at[u], sems.at[3 + u]) for u in range(2)]
    cp_c = pltpu.make_async_copy(c_hbm.at[0], c_s, sems.at[5])
    cp_wo = pltpu.make_async_copy(woT_hbm, woT_s, sems.at[6])

    def cp_kv(i, which, u):
        src = (wk_hbm, wv_hbm)[which]
        dst = (wk_r, wv_r)[which]
        return pltpu.make_async_copy(src.at[pl.ds(i * 1024, 1024), pl.ds(128 * u, 128)], dst.at[u, i], csems.at[i, 2 * which + u])

    NX = 4
    XW = S // NX
    cp_x = [pltpu.make_async_copy(xT_hbm.at[0, :, pl.ds(i * XW, XW)], xT_s.at[:, pl.ds(i * XW, XW)], xsems.at[i]) for i in range(NX)]
    cp_wqkv.start(); cp_x[0].start()

    def start_kv(lo, hi):
        for i in range(lo, hi):
            for w in range(2):
                for u in range(2):
                    cp_kv(i, w, u).start()

    with jax.named_scope("w_wqkv"):
        cp_wqkv.wait()
    for i in range(1, NX):
        cp_x[i].start()
    cp_bwo.start()
    for u in range(11):
        w = min(128, 1344 - u * 128)
        wqkvT_s[u*128:u*128+w, :] = wqkv_s[:, u*128:u*128+w].astype(F32).T.astype(BF)
    wqkvT_s[1344:1360, :] = jnp.broadcast_to(gw_ref[...].reshape(1, M), (16, M)).astype(BF)
    with jax.named_scope("w_x"):
        cp_x[0].wait()
    cp_wq[0].start(); cp_wq[1].start()
    CH = 512
    NC = S // CH
    kv_s[...] = jnp.zeros_like(kv_s)

    def p1body(i, _, deint):
        @pl.when(i == 1)
        def _():
            cp_bwo.wait()
            bwoT_s[...] = bwo_s[...].astype(F32).T.astype(BF)
        for n in range(1, NX):
            @pl.when(i == n * (XW // CH))
            def _():
                cp_x[n].wait()
        @pl.when(i == NC * 3 // 4)
        def _():
            start_kv(4, 8)
        cols = pl.ds(pl.multiple_of(i * CH, CH), CH)
        xb = xT_s[:, cols]
        t = jnp.dot(wqkvT_s[0:896, :], xb, preferred_element_type=F32)
        ph = (jnp.where(t > 0, t + 1.0, jnp.exp(t)) + 1e-6).astype(BF)
        pqT_s[:, cols] = ph[0:448]
        vg = jnp.dot(wqkvT_s[896:1360, :], xb, preferred_element_type=F32)
        vT = vg[0:448].astype(BF)
        g_s[:, cols] = 1.0 / (1.0 + jnp.exp(-vg[448:456]))
        ones = jnp.ones((16, CH), BF)
        for r, (lo, hi) in enumerate(ERANGE):
            dn = min(128, 448 - 128 * r)
            lhs = jnp.concatenate([vT[lo:hi], ones], axis=0)
            kk = lax.dot_general(lhs, ph[448 + 128 * r:448 + 128 * r + dn], NT, preferred_element_type=F32)
            kv_s[r, 0:hi - lo + 16, 0:dn] += kk
        xa_s[cols, :] = xb.astype(F32).T.astype(BF)
        acc_s[:, cols] = jnp.zeros((M, CH), F32)
        if deint:
            per = 8 // NC
            for e in range(per):
                mc = (i - NC // 2) * per + e
                for u in range(2):
                    sub = wq_r.at[u, pl.ds(pl.multiple_of(mc * 1792, 1792), 1792)]
                    for j in range(8):
                        _deint_piece(wq_d, sub, u, j, pl.multiple_of(mc * 112, 16), 112)
        return _
    with jax.named_scope("pass1"):
        lax.fori_loop(0, NC // 2, functools.partial(p1body, deint=False), None)
    with jax.named_scope("w_wq"):
        cp_wq[0].wait(); cp_wq[1].wait()
    start_kv(0, 4)
    with jax.named_scope("pass1b"):
        lax.fori_loop(NC // 2, NC, functools.partial(p1body, deint=True), None)

    for r, (lo, hi) in enumerate(ERANGE):
        dn = min(128, 448 - 128 * r)
        n = hi - lo
        e = lax.broadcasted_iota(jnp.int32, (n, dn), 0) + lo
        d = lax.broadcasted_iota(jnp.int32, (n, dn), 1) + 128 * r
        same = ((e * 2341) >> 16) == ((d * 2341) >> 16)
        kvm_s[r, 0:n, 0:dn] = jnp.where(same, kv_s[r, 0:n, 0:dn], 0.0).astype(BF)
        zrow = kv_s[r, n:n + 8, 0:dn]
        zm_s[r, 0:n, 0:dn] = jnp.where(same, jnp.tile(zrow, (n // 8, 1)), 0.0).astype(BF)

    def assemble(parts):
        out = []
        bounds = sorted(set([0, 448] + [x for rg in ERANGE for x in rg]))
        for a, b in zip(bounds[:-1], bounds[1:]):
            acc = None
            for r, (lo, hi) in enumerate(ERANGE):
                if lo <= a and b <= hi:
                    p = parts[r][a - lo:b - lo]
                    acc = p if acc is None else acc + p
            out.append(acc)
        return jnp.concatenate(out, axis=0)

    def numden(i):
        cols = pl.ds(pl.multiple_of(i * CH, CH), CH)
        nums = []; dens = []
        for r, (lo, hi) in enumerate(ERANGE):
            dn = min(128, 448 - 128 * r)
            pq = pqT_s[128 * r:128 * r + dn, cols]
            nums.append(jnp.dot(kvm_s[r, 0:hi - lo, 0:dn], pq, preferred_element_type=F32))
            dens.append(jnp.dot(zm_s[r, 0:hi - lo, 0:dn], pq, preferred_element_type=F32))
        return (assemble(nums) / (assemble(dens) + 1e-6)).astype(BF)

    CH = 256
    NC = S // CH
    start_kv(8, 12)

    def p2body(i, _):
        @pl.when(i == 2)
        def _():
            start_kv(12, 16)
        oa = numden(2 * i)
        ob = numden(2 * i + 1)
        for n, o in enumerate((oa, ob)):
            cols = pl.ds(pl.multiple_of((2 * i + n) * CH, CH), CH)
            bT_s[:, cols] = (1.0 - g_s[0:1, cols]) * jnp.dot(bwoT_s[...], o, preferred_element_type=F32)
        return _
    with jax.named_scope("pass2"):
        lax.fori_loop(0, NC // 2, p2body, None)

    def qbody(h, _):
        m0 = pl.multiple_of(h * 64, 64)
        wq = wq_d[h]
        for i in range(S // 256):
            rows = slice(i * 256, (i + 1) * 256)
            q_all[h, rows, :] = (jnp.dot(xa_s[rows, :], wq, preferred_element_type=F32) * (LOG2E / 16.0)).astype(BF)
            for u in range(2):
                _deint_piece(wk_d, wk_r.at[u, h], u, i, m0, 64)
                _deint_piece(wv_d, wv_r.at[u, h], u, i, m0, 64)
        return _
    for half in range(2):
        with jax.named_scope("w_kv%d" % half):
            for i in range(half * 8, half * 8 + 8):
                for w in range(2):
                    for u in range(2):
                        cp_kv(i, w, u).wait()
        (cp_c, cp_wo)[half].start()
        with jax.named_scope("qloop%d" % half):
            lax.fori_loop(half * 8, half * 8 + 8, qbody, None, unroll=4)

    with jax.named_scope("w_c"):
        cp_c.wait(); cp_wo.wait()

    def outproj(hh, t, ctx):
        acc_s[:, t * BQ:(t + 1) * BQ] += lax.dot_general(woT_s[hh], ctx, NT, preferred_element_type=F32)

    def kproj(hh, i):
        rows = slice(i * BQ, (i + 1) * BQ)
        k_s[rows, :] = jnp.dot(c_s[rows, :], wk_d[hh], preferred_element_type=F32).astype(BF)

    def vproj(hh, i):
        rows = slice(i * BQ, (i + 1) * BQ)
        v_s[rows, :] = jnp.dot(c_s[rows, :], wv_d[hh], preferred_element_type=F32).astype(BF)

    def hbody(h, _):
        HB = BQ // 2
        tri = lax.broadcasted_iota(jnp.int32, (HB, HB), 1) <= lax.broadcasted_iota(jnp.int32, (HB, HB), 0)

        def qk(t):
            q = q_all[h, t * BQ:(t + 1) * BQ, :]
            m = None
            sl = t % 2
            for j in range(t):
                s = lax.dot_general(q, k_s[j * BQ:(j + 1) * BQ, :], NT, preferred_element_type=F32)
                s_s[sl, :, j * BQ:(j + 1) * BQ] = s
                for u in range(BQ // 128):
                    mm = s[:, u * 128:(u + 1) * 128]
                    m = mm if m is None else jnp.maximum(m, mm)
            c0 = t * BQ
            if DIAG == 0:
                s = lax.dot_general(q, k_s[c0:c0 + BQ, :], NT, preferred_element_type=F32)
                r = lax.broadcasted_iota(jnp.int32, (BQ, BQ), 1)
                c = lax.broadcasted_iota(jnp.int32, (BQ, BQ), 0)
                s = jnp.where(r <= c, s, -1e9)
                s_s[sl, :, c0:c0 + BQ] = s
                for u in range(BQ // 128):
                    mm = s[:, u * 128:(u + 1) * 128]
                    m = mm if m is None else jnp.maximum(m, mm)
                return jnp.max(m, axis=1, keepdims=True)
            else:
                sa = lax.dot_general(q, k_s[c0:c0 + HB, :], NT, preferred_element_type=F32)
                sb = lax.dot_general(q[HB:], k_s[c0 + HB:c0 + BQ, :], NT, preferred_element_type=F32)
                sa = jnp.concatenate([jnp.where(tri, sa[:HB], -1e9), sa[HB:]], axis=0)
                sb = jnp.where(tri, sb, -1e9)
                s_s[sl, :, c0:c0 + HB] = sa
                s_s[sl, HB:, c0 + HB:c0 + BQ] = sb
                m = sa if m is None else jnp.maximum(m, sa)
                m = jnp.concatenate([m[:HB], jnp.maximum(m[HB:], sb)], axis=0)
                return jnp.max(m, axis=1, keepdims=True)

        def pv(t, m):
            acc = None; l = None
            sl = t % 2
            prev = []
            def paced(mm):
                if PACE and len(prev) >= PACE:
                    a = prev[-PACE][:, 0:1]
                    return jnp.maximum(mm, jnp.minimum(mm, a))
                return mm
            def psum(p):
                pb = p.astype(BF)
                return pb, (pb.astype(F32) if LBF else p)
            for j in range(t):
                p = jnp.exp2(s_s[sl, :, j * BQ:(j + 1) * BQ] - paced(m))
                pb, p = psum(p)
                for u in range(BQ // 128):
                    ll = p[:, u * 128:(u + 1) * 128]
                    l = ll if l is None else l + ll
                a = jnp.dot(pb, v_s[j * BQ:(j + 1) * BQ, :], preferred_element_type=F32)
                prev.append(a)
                acc = a if acc is None else acc + a
            c0 = t * BQ
            mm = paced(m)
            pa, paf = psum(jnp.exp2(s_s[sl, :, c0:c0 + HB] - mm))
            pb, pbf = psum(jnp.exp2(s_s[sl, HB:, c0 + HB:c0 + BQ] - mm[HB:]))
            l = paf if l is None else l + paf
            l = jnp.concatenate([l[:HB], l[HB:] + pbf], axis=0)
            a = jnp.dot(pa, v_s[c0:c0 + HB, :], preferred_element_type=F32)
            acc = a if acc is None else acc + a
            a2 = jnp.dot(pb, v_s[c0 + HB:c0 + BQ, :], preferred_element_type=F32)
            acc = jnp.concatenate([acc[:HB], acc[HB:] + a2], axis=0)
            l = jnp.sum(l, axis=1, keepdims=True)
            return (acc * (1.0 / l)).astype(BF)

        hn = jnp.minimum(h + 1, H - 1)
        for t in range(NB):
            m = qk(t)
            if t + 1 < NB:
                kproj(h, t + 1)
            else:
                kproj(hn, 0)
            ctx = pv(t, m)
            if t + 1 < NB:
                vproj(h, t + 1)
            else:
                vproj(hn, 0)
            outproj(h, t, ctx)
        return _
    with jax.named_scope("hloop"):
        kproj(0, 0); vproj(0, 0)
        lax.fori_loop(0, H, hbody, None)

    NO = 4
    W = S // NO
    ocp = []
    for i in range(NO):
        cols = slice(i * W, (i + 1) * W)
        out_s[:, cols] = (g_s[0:1, cols] * acc_s[:, cols] + bT_s[:, cols]).astype(out_s.dtype)
        cp = pltpu.make_async_copy(out_s.at[:, pl.ds(i * W, W)], out_hbm.at[0, :, pl.ds(i * W, W)], osems.at[i])
        cp.start()
        ocp.append(cp)
    with jax.named_scope("w_out"):
        for cp in ocp:
            cp.wait()


@jax.jit
def pallas_gated_mix__compressed_kv_cla__linear_attn_block__prompt_kernel(
    A_x, A_c_kv, A_w_q, A_w_uk, A_w_uv, A_w_o, B_x, B_wqkv, B_wo, gate_w,
):
    B, S, M = A_x.shape
    Dc = A_c_kv.shape[2]
    H, D = A_w_q.shape[1], A_w_q.shape[2]
    anyspec = pl.BlockSpec(memory_space=pl.ANY)
    wq = A_w_q.reshape(M * H, D)
    wk = A_w_uk.reshape(Dc * H, D)
    wv = A_w_uv.reshape(Dc * H, D)
    outT = pl.pallas_call(
        kernel,
        in_specs=[anyspec] * 8 + [pl.BlockSpec(memory_space=pltpu.VMEM)],
        out_specs=anyspec,
        out_shape=jax.ShapeDtypeStruct((B, M, S), BF),
        scratch_shapes=[
            pltpu.VMEM((M, S), BF), pltpu.VMEM((S, Dc), BF), pltpu.VMEM((2, M * H, 128), BF),
            pltpu.VMEM((2, H, Dc, 128), BF), pltpu.VMEM((2, H, Dc, 128), BF), pltpu.VMEM((H, M, D), BF),
            pltpu.VMEM((M, 3 * M), BF), pltpu.VMEM((M, M), BF), pltpu.VMEM((M, S), BF),
            pltpu.VMEM((H, S, D), BF), pltpu.VMEM((S, D), BF), pltpu.VMEM((S, D), BF),
            pltpu.VMEM((2, BQ, S), F32), pltpu.VMEM((M, S), F32), pltpu.VMEM((M, S), F32), pltpu.VMEM((8, S), F32),
            pltpu.VMEM((H, M, D), BF), pltpu.VMEM((H, Dc, D), BF), pltpu.VMEM((H, Dc, D), BF),
            pltpu.VMEM((S, M), BF), pltpu.VMEM((3 * M + 16, M), BF), pltpu.VMEM((M, S), BF), pltpu.VMEM((M, M), BF),
            pltpu.VMEM((4, 192, 128), F32), pltpu.VMEM((4, 176, 128), BF), pltpu.VMEM((4, 176, 128), BF),
            pltpu.SemaphoreType.DMA((7,)), pltpu.SemaphoreType.DMA((H, 4)), pltpu.SemaphoreType.DMA((4,)), pltpu.SemaphoreType.DMA((4,)),
        ],
        compiler_params=pltpu.CompilerParams(vmem_limit_bytes=120 * 2**20),
    )(A_x.transpose(0, 2, 1), A_c_kv, wq, wk, wv, A_w_o.transpose(0, 2, 1), B_wqkv, B_wo, gate_w)
    return outT.transpose(0, 2, 1)
```
